```python
import jax
import jax.numpy as jnp

def _softmax(x, axis=-1):
    return jax.nn.softmax(x, axis=axis)
def _gelu(x):
    return jax.nn.gelu(x, approximate=True)
def _silu(x):
    return jax.nn.silu(x)
def _sigmoid(x):
    return jax.nn.sigmoid(x)
def _layernorm(x, axis=-1, eps=1e-5):
    m = jnp.mean(x, axis=axis, keepdims=True)
    v = jnp.var(x, axis=axis, keepdims=True)
    return (x - m) / jnp.sqrt(v + eps)
def _scatter_add(tgt, idx, src, axis=0):
    return tgt.at[idx].add(src)
def _segment_sum(src, seg, n):
    return jax.ops.segment_sum(src, seg, n)
class _Rng:
    def __init__(self, key):
        self._k = key
    def _next(self):
        self._k, sub = jax.random.split(self._k)
        return sub
    def normal(self, shape):
        return jax.random.normal(self._next(), shape, dtype=jnp.bfloat16)
    def randint(self, lo, hi, shape):
        return jax.random.randint(self._next(), shape, lo, hi, dtype=jnp.int32)
    def uniform(self, shape, lo=0.0, hi=1.0):
        return jax.random.uniform(self._next(), shape, jnp.bfloat16, lo, hi)
    def permutation(self, n):
        return jax.random.permutation(self._next(), n)


kernel_name = 'gated_mix__sliding_local_dilated__glu_gated_reglu__prompt'

def setup_inputs():
    _rng = _Rng(jax.random.key(int.from_bytes(__import__("os").urandom(4), "little")))
    _w = (lambda a: (lambda t: t.astype(jnp.bfloat16) if jnp.issubdtype(t.dtype, jnp.floating) else t)(jnp.asarray(a)))
    def _A_setup():
        B, S, D = 1, 2048, 1024
        return {
            "x": _w((lambda *s: _rng.normal(s) * 0.05)(B, S, D)),
            "wqkv": _w((lambda *s: _rng.normal(s) * 0.05)(D, 3 * D)),
            "wo": _w((lambda *s: _rng.normal(s) * 0.05)(D, D)),
        }
    _A_in = _A_setup()

    def _B_setup():
        B, S, D, F = 1, 2048, 1024, 3584
        return {
            "x": _w((lambda *s: _rng.normal(s) * 0.05)(B, S, D)),
            "W_gate": _w((lambda *s: _rng.normal(s) * 0.05)(D, F) * (2.0 / D) ** 0.5),
            "W_up": _w((lambda *s: _rng.normal(s) * 0.05)(D, F) * (2.0 / D) ** 0.5),
            "W_down": _w((lambda *s: _rng.normal(s) * 0.05)(F, D) * (1.0 / F) ** 0.5),
        }
    _B_in = _B_setup()

    return {
        "A_x": _A_in["x"],
        "A_wqkv": _A_in["wqkv"],
        "A_wo": _A_in["wo"],
        "B_x": _B_in["x"],
        "B_W_gate": _B_in["W_gate"],
        "B_W_up": _B_in["W_up"],
        "B_W_down": _B_in["W_down"],
        "gate_w": _w((lambda *s: _rng.normal(s) * 0.05)(1024)),
    }

def reference(A_x, A_wqkv, A_wo, B_x, B_W_gate, B_W_up, B_W_down, gate_w):
    def _A_ref(x, wqkv, wo):
        B, S, D = x.shape
        H = 32; Dh = D // H
        W, dil = 8, 2
        qkv = (lambda x, *d: x.transpose(*d))((x @ wqkv).reshape(B, S, 3, H, Dh), 2, 0, 3, 1, 4)
        q, k, v = qkv[0], qkv[1], qkv[2]
        scale = Dh ** -0.5
        pos = jnp.arange(S)
        off = jnp.arange(W) * dil
        idx = pos[:, None] - off[None, :]
        mask = idx >= 0
        idx_c = jnp.where(mask, idx, 0).reshape(-1)
        kg = k[:, :, idx_c, :].reshape(B, H, S, W, Dh)
        vg = v[:, :, idx_c, :].reshape(B, H, S, W, Dh)
        logits = jnp.einsum("bhsd,bhswd->bhsw", q, kg) * scale
        logits = jnp.where(mask[None, None, :, :], logits, -1e9)
        attn = _softmax(logits, axis=-1)
        o = jnp.einsum("bhsw,bhswd->bhsd", attn, vg)
        return (lambda x, *d: x.transpose(*d))(o, 0, 2, 1, 3).reshape(B, S, D) @ wo

    def _B_ref(x, W_gate, W_up, W_down):
        gate = jnp.einsum("bsd,df->bsf", x, W_gate)
        up = jnp.einsum("bsd,df->bsf", x, W_up)
        gate = gate * (lambda x, dt: x.astype(dt))(gate > 0, gate.dtype)
        h = gate * up
        return jnp.einsum("bsf,fd->bsd", h, W_down)

    x = A_x
    g = _sigmoid((x * gate_w).sum(-1, keepdims=True))
    a = _A_ref(x, A_wqkv, A_wo)
    b = _B_ref(x, B_W_gate, B_W_up, B_W_down)
    return g * a + (1 - g) * b
```

```python
import functools

import jax
import jax.numpy as jnp
import numpy as np
from jax import lax
import jax.experimental.pallas as pl
import jax.experimental.pallas.tpu as pltpu

S, D, F = 2048, 1024, 3584
H, DH, W, DIL = 32, 32, 8, 2
HALO = 16
NT = D // 128

T = 512
FC = 896
NC = F // FC
AR = T // NC

_F32 = jnp.float32
_BF16 = jnp.bfloat16
_SCALE = float(DH ** -0.5)


def _nt_dot(a, b):
    return lax.dot_general(a, b, (((1,), (1,)), ((), ())), preferred_element_type=_F32)


def _dot(a, b):
    return jnp.dot(a, b, preferred_element_type=_F32)


def _kernel(x_ref, gw_ref, wqkv_hbm, wo_hbm, wg_hbm, wu_hbm, wd_hbm, out_ref,
            wqkv_raw, wo_raw, tmp_t, wqkv_p, wo_p, wg, wu, wd,
            q_s, k_s, v_s, o_s, acc, sems):
    i = pl.program_id(0)

    def cp_g(c):
        return pltpu.make_async_copy(wg_hbm.at[:, pl.ds(c * FC, FC)], wg.at[c], sems.at[3 * c])

    def cp_u(c):
        return pltpu.make_async_copy(wu_hbm.at[:, pl.ds(c * FC, FC)], wu.at[c], sems.at[3 * c + 1])

    def cp_d(c):
        return pltpu.make_async_copy(wd_hbm.at[pl.ds(c * FC, FC), :], wd.at[c], sems.at[3 * c + 2])

    cp_qkv = pltpu.make_async_copy(wqkv_hbm, wqkv_raw, sems.at[3 * NC])
    cp_o = pltpu.make_async_copy(wo_hbm, wo_raw, sems.at[3 * NC + 1])

    @pl.when(i == 0)
    def _():
        cp_qkv.start()
        cp_o.start()
        for c in range(NC):
            cp_g(c).start()
            cp_u(c).start()
            cp_d(c).start()
        k_s[:, pl.ds(0, HALO), :] = jnp.zeros((NT, HALO, 128), _F32)
        v_s[:, pl.ds(0, HALO), :] = jnp.zeros((NT, HALO, 128), _F32)
        cp_qkv.wait()
        def permute_rows(dst, base):
            for kt in range(NT):
                for j in range(NT):
                    for dd in range(4):
                        rows = tmp_t[kt, pl.ds(j * 4 + dd, H, stride=DH), :]
                        dst[pl.ds(base + j * 128 + dd * 32, 32), pl.ds(kt * 128, 128)] = rows.astype(_BF16)

        for m in range(3):
            for kt in range(NT):
                blk = wqkv_raw[pl.ds(kt * 128, 128), pl.ds(m * D, D)].astype(_F32)
                tmp_t[kt] = blk.T
            permute_rows(wqkv_p, m * D)
        cp_o.wait()
        for kt in range(NT):
            tmp_t[kt] = wo_raw[:, pl.ds(kt * 128, 128)].astype(_F32)
        permute_rows(wo_p, 0)

    @pl.when(i > 0)
    def _():
        k_s[:, pl.ds(0, HALO), :] = k_s[:, pl.ds(T, HALO), :]
        v_s[:, pl.ds(0, HALO), :] = v_s[:, pl.ds(T, HALO), :]

    x = x_ref[...]
    qkv = _nt_dot(x, wqkv_p[...])
    for j in range(NT):
        q_s[j] = qkv[:, j * 128:(j + 1) * 128]
        k_s[j, pl.ds(HALO, T), :] = qkv[:, D + j * 128:D + (j + 1) * 128]
        v_s[j, pl.ds(HALO, T), :] = qkv[:, 2 * D + j * 128:2 * D + (j + 1) * 128]

    def attn(r0, first):
        logits = []
        for w in range(W):
            p = None
            for j in range(NT):
                t = q_s[j, pl.ds(r0, AR), :] * k_s[j, pl.ds(r0 + HALO - DIL * w, AR), :]
                p = t if p is None else p + t
            p = p + pltpu.roll(p, 64, 1)
            p = p + pltpu.roll(p, 32, 1)
            p = p * _SCALE
            if first and w > 0:
                pos = lax.broadcasted_iota(jnp.int32, (AR, 128), 0) + (i * T + r0)
                p = jnp.where(pos >= DIL * w, p, -1e9)
            logits.append(p)
        m = functools.reduce(jnp.maximum, logits)
        es = [jnp.exp(l - m) for l in logits]
        inv = 1.0 / functools.reduce(jnp.add, es)
        ps = [e * inv for e in es]
        for j in range(NT):
            o = None
            for w in range(W):
                t = ps[w] * v_s[j, pl.ds(r0 + HALO - DIL * w, AR), :]
                o = t if o is None else o + t
            o_s[pl.ds(r0, AR), pl.ds(j * 128, 128)] = o.astype(_BF16)

    for c in range(NC):
        @pl.when(i == 0)
        def _():
            cp_g(c).wait()
            cp_u(c).wait()
            cp_d(c).wait()
        attn(c * AR, c == 0)
        gate = _dot(x, wg[c])
        up = _dot(x, wu[c])
        h = (jnp.maximum(gate, 0.0) * up).astype(_BF16)
        b = _dot(h, wd[c])
        if c == 0:
            acc[...] = b
        elif c < NC - 1:
            acc[...] += b
        else:
            a = _dot(o_s[...], wo_p[...])
            g = jax.nn.sigmoid(jnp.sum(x.astype(_F32) * gw_ref[...].astype(_F32), axis=-1, keepdims=True))
            out_ref[...] = (g * a + (1.0 - g) * (acc[...] + b)).astype(out_ref.dtype)


@jax.jit
def pallas_gated_mix__sliding_local_dilated__glu_gated_reglu__prompt_kernel(
        A_x: jax.Array,
        A_wqkv: jax.Array,
        A_wo: jax.Array,
        B_x: jax.Array,
        B_W_gate: jax.Array,
        B_W_up: jax.Array,
        B_W_down: jax.Array,
        gate_w: jax.Array,
):
    del B_x
    x = A_x.reshape(S, D)
    gw = gate_w.reshape(1, D)
    any_spec = pl.BlockSpec(memory_space=pl.ANY)
    out = pl.pallas_call(
        _kernel,
        grid=(S // T,),
        in_specs=[pl.BlockSpec((T, D), lambda i: (i, 0)),
                  pl.BlockSpec((1, D), lambda i: (0, 0)),
                  any_spec, any_spec, any_spec, any_spec, any_spec],
        out_specs=pl.BlockSpec((T, D), lambda i: (i, 0)),
        out_shape=jax.ShapeDtypeStruct((S, D), A_x.dtype),
        scratch_shapes=[
            pltpu.VMEM((D, 3 * D), _BF16),
            pltpu.VMEM((D, D), _BF16),
            pltpu.VMEM((NT, D, 128), _F32),
            pltpu.VMEM((3 * D, D), _BF16),
            pltpu.VMEM((D, D), _BF16),
            pltpu.VMEM((NC, D, FC), _BF16),
            pltpu.VMEM((NC, D, FC), _BF16),
            pltpu.VMEM((NC, FC, D), _BF16),
            pltpu.VMEM((NT, T, 128), _F32),
            pltpu.VMEM((NT, T + HALO, 128), _F32),
            pltpu.VMEM((NT, T + HALO, 128), _F32),
            pltpu.VMEM((T, D), _BF16),
            pltpu.VMEM((T, D), _F32),
            pltpu.SemaphoreType.DMA((3 * NC + 2,)),
        ],
        compiler_params=pltpu.CompilerParams(
            dimension_semantics=("arbitrary",),
            vmem_limit_bytes=110 * 1024 * 1024),
    )(x, gw, A_wqkv, A_wo, B_W_gate, B_W_up, B_W_down)
    return out.reshape(1, S, D)
```

```python
import functools

import jax
import jax.numpy as jnp
import numpy as np
from jax import lax
import jax.experimental.pallas as pl
import jax.experimental.pallas.tpu as pltpu

S, D, F = 2048, 1024, 3584
H, DH, W, DIL = 32, 32, 8, 2
HALO = 16
NT = D // 128

T = S
PREP_AT = 1
OC = 128
ATT_AT = 3
PROJ_AT = 2
FC = 512
NC = F // FC
AR = 128

_F32 = jnp.float32
_BF16 = jnp.bfloat16
_SCALE = float(DH ** -0.5)


def _nt_dot(a, b):
    return lax.dot_general(a, b, (((1,), (1,)), ((), ())), preferred_element_type=_F32)


def _dot(a, b):
    return jnp.dot(a, b, preferred_element_type=_F32)


def _kernel(x_hbm, gw_ref, wqkv_hbm, wo_hbm, wg_hbm, wu_hbm, wd_hbm, out_hbm,
            x_s, out_s, wqkv_raw, wo_raw, tmp_t, wqkv_p, wo_p, wg, wu, wd,
            q_s, k_s, v_s, o_s, acc, sems):
    def cp_g(c):
        return pltpu.make_async_copy(wg_hbm.at[:, pl.ds(c * FC, FC)], wg.at[c % 2], sems.at[3 * c])

    def cp_u(c):
        return pltpu.make_async_copy(wu_hbm.at[:, pl.ds(c * FC, FC)], wu.at[c % 2], sems.at[3 * c + 1])

    def cp_d(c):
        return pltpu.make_async_copy(wd_hbm.at[pl.ds(c * FC, FC), :], wd.at[c % 2], sems.at[3 * c + 2])

    cp_qkv = pltpu.make_async_copy(wqkv_hbm, wqkv_raw, sems.at[3 * NC])
    cp_o = pltpu.make_async_copy(wo_hbm, wo_raw, sems.at[3 * NC + 1])
    cp_x = pltpu.make_async_copy(x_hbm, x_s, sems.at[3 * NC + 2])

    def cp_out(n):
        cs = pl.ds(n * OC, OC)
        return pltpu.make_async_copy(out_s.at[:, cs], out_hbm.at[:, cs], sems.at[3 * NC + 3 + n])

    cp_x.start()
    for c in range(2):
        cp_g(c).start()
        cp_u(c).start()
        cp_d(c).start()
    cp_qkv.start()
    cp_o.start()
    k_s[:, pl.ds(0, HALO), :] = jnp.zeros((NT, HALO, 128), _F32)
    v_s[:, pl.ds(0, HALO), :] = jnp.zeros((NT, HALO, 128), _F32)

    def permute_rows(dst, base):
        for kt in range(NT):
            for j in range(NT):
                for dd in range(4):
                    rows = tmp_t[kt, pl.ds(j * 4 + dd, H, stride=DH), :]
                    dst[pl.ds(base + j * 128 + dd * 32, 32), pl.ds(kt * 128, 128)] = rows.astype(_BF16)

    def prep():
        cp_qkv.wait()
        cp_o.wait()
        for m in range(3):
            for kt in range(NT):
                blk = wqkv_raw[pl.ds(kt * 128, 128), pl.ds(m * D, D)].astype(_F32)
                tmp_t[kt] = blk.T
            permute_rows(wqkv_p, m * D)
        for kt in range(NT):
            tmp_t[kt] = wo_raw[:, pl.ds(kt * 128, 128)].astype(_F32)
        permute_rows(wo_p, 0)

    def project():
        for m, dst, off in ((0, q_s, 0), (1, k_s, HALO), (2, v_s, HALO)):
            y = _nt_dot(x_s[...], wqkv_p[pl.ds(m * D, D), :])
            for j in range(NT):
                dst[j, pl.ds(off, S), :] = y[:, j * 128:(j + 1) * 128]

    def attn(r0):
        logits = []
        for w in range(W):
            p = None
            for j in range(NT):
                t = q_s[j, pl.ds(r0, AR), :] * k_s[j, pl.ds(r0 + HALO - DIL * w, AR), :]
                p = t if p is None else p + t
            p = p + pltpu.roll(p, 64, 1)
            p = p + pltpu.roll(p, 32, 1)
            p = p * _SCALE
            if r0 < DIL * w:
                pos = lax.broadcasted_iota(jnp.int32, (AR, 128), 0) + r0
                p = jnp.where(pos >= DIL * w, p, -1e9)
            logits.append(p)
        m = functools.reduce(jnp.maximum, logits)
        es = [jnp.exp(l - m) for l in logits]
        inv = 1.0 / functools.reduce(jnp.add, es)
        ps = [e * inv for e in es]
        for j in range(NT):
            o = None
            for w in range(W):
                t = ps[w] * v_s[j, pl.ds(r0 + HALO - DIL * w, AR), :]
                o = t if o is None else o + t
            o_s[pl.ds(r0, AR), pl.ds(j * 128, 128)] = o.astype(_BF16)

    cp_x.wait()
    for c in range(NC):
        cp_g(c).wait()
        cp_u(c).wait()
        if c > 0:
            cp_d(c).wait()
        if c == PREP_AT:
            prep()
        if c == PROJ_AT:
            project()
        if c >= ATT_AT:
            n = S // AR // (NC - ATT_AT)
            for t in range(n):
                attn(((c - ATT_AT) * n + t) * AR)
        x = x_s[...]
        gate = _dot(x, wg[c % 2])
        up = _dot(x, wu[c % 2])
        h = (jnp.maximum(gate, 0.0) * up).astype(_BF16)
        if c == 0:
            cp_d(c).wait()
        if c < NC - 1:
            b = _dot(h, wd[c % 2])
        if c + 2 < NC:
            cp_g(c + 2).start()
            cp_u(c + 2).start()
            cp_d(c + 2).start()
        if c == 0:
            acc[...] = b
        elif c < NC - 1:
            acc[...] += b
        else:
            g = jax.nn.sigmoid(jnp.sum(x.astype(_F32) * gw_ref[...].astype(_F32), axis=-1, keepdims=True))
            for n in range(D // OC):
                cs = pl.ds(n * OC, OC)
                b = _dot(h, wd[c % 2, :, cs])
                a = _dot(o_s[...], wo_p[:, cs])
                out_s[:, cs] = (g * a + (1.0 - g) * (acc[:, cs] + b)).astype(out_s.dtype)
                cp_out(n).start()
    for n in range(D // OC):
        cp_out(n).wait()


@jax.jit
def pallas_gated_mix__sliding_local_dilated__glu_gated_reglu__prompt_kernel(
        A_x: jax.Array,
        A_wqkv: jax.Array,
        A_wo: jax.Array,
        B_x: jax.Array,
        B_W_gate: jax.Array,
        B_W_up: jax.Array,
        B_W_down: jax.Array,
        gate_w: jax.Array,
):
    del B_x
    x = A_x.reshape(S, D)
    gw = gate_w.reshape(1, D)
    any_spec = pl.BlockSpec(memory_space=pl.ANY)
    out = pl.pallas_call(
        _kernel,
        in_specs=[any_spec, pl.BlockSpec(memory_space=pltpu.VMEM),
                  any_spec, any_spec, any_spec, any_spec, any_spec],
        out_specs=any_spec,
        out_shape=jax.ShapeDtypeStruct((S, D), A_x.dtype),
        scratch_shapes=[
            pltpu.VMEM((S, D), _BF16),
            pltpu.VMEM((S, D), A_x.dtype),
            pltpu.VMEM((D, 3 * D), _BF16),
            pltpu.VMEM((D, D), _BF16),
            pltpu.VMEM((NT, D, 128), _F32),
            pltpu.VMEM((3 * D, D), _BF16),
            pltpu.VMEM((D, D), _BF16),
            pltpu.VMEM((2, D, FC), _BF16),
            pltpu.VMEM((2, D, FC), _BF16),
            pltpu.VMEM((2, FC, D), _BF16),
            pltpu.VMEM((NT, T, 128), _F32),
            pltpu.VMEM((NT, T + HALO, 128), _F32),
            pltpu.VMEM((NT, T + HALO, 128), _F32),
            pltpu.VMEM((T, D), _BF16),
            pltpu.VMEM((T, D), _F32),
            pltpu.SemaphoreType.DMA((3 * NC + 3 + D // OC,)),
        ],
        compiler_params=pltpu.CompilerParams(
            vmem_limit_bytes=120 * 1024 * 1024),
    )(x, gw, A_wqkv, A_wo, B_W_gate, B_W_up, B_W_down)
    return out.reshape(1, S, D)
```
